```python
import os as _os
_os.environ.setdefault("JAX_PLATFORMS", "cpu")
import jax
import jax.numpy as jnp

def _softmax(x, axis=-1):
    return jax.nn.softmax(x, axis=axis)
def _gelu(x):
    return jax.nn.gelu(x, approximate=True)
def _silu(x):
    return jax.nn.silu(x)
def _sigmoid(x):
    return jax.nn.sigmoid(x)
def _layernorm(x, axis=-1, eps=1e-5):
    m = jnp.mean(x, axis=axis, keepdims=True)
    v = jnp.var(x, axis=axis, keepdims=True)
    return (x - m) / jnp.sqrt(v + eps)
def _scatter_add(tgt, idx, src, axis=0):
    return tgt.at[idx].add(src)
def _segment_sum(src, seg, n):
    return jax.ops.segment_sum(src, seg, n)
class _Rng:
    def __init__(self, key):
        self._k = key
    def _next(self):
        self._k, sub = jax.random.split(self._k)
        return sub
    def normal(self, shape):
        return jax.random.normal(self._next(), shape, dtype=jnp.bfloat16)
    def randint(self, lo, hi, shape):
        return jax.random.randint(self._next(), shape, lo, hi, dtype=jnp.int32)
    def uniform(self, shape, lo=0.0, hi=1.0):
        return jax.random.uniform(self._next(), shape, jnp.bfloat16, lo, hi)
    def permutation(self, n):
        return jax.random.permutation(self._next(), n)


kernel_name = 'concat_heads__mha_block_cached__mha_block_cached__near_ridge'

def setup_inputs():
    _rng = _Rng(jax.random.key(int.from_bytes(__import__("os").urandom(4), "little")))
    _w = (lambda a: (lambda t: t.astype(jnp.bfloat16) if jnp.issubdtype(t.dtype, jnp.floating) else t)(jnp.asarray(a)))
    def _A_setup():
        B, Sq, D = 8, 144, 640
        H, Sk, Dh = 32, 512, 128
        return {
            "x": _w((lambda *s: _rng.normal(s) * 0.8)(B, Sq, D)),
            "k_cache": _w((lambda *s: _rng.normal(s) * 0.8)(B, H, Sk, Dh)),
            "v_cache": _w((lambda *s: _rng.normal(s) * 0.05)(B, H, Sk, Dh)),
            "wq": _w((lambda *s: _rng.normal(s) * 0.8)(D, H * Dh) * (D ** -0.5)),
            "wo": _w((lambda *s: _rng.normal(s) * 0.05)(H * Dh, D) * ((H * Dh) ** -0.5)),
        }
    _A_in = _A_setup()

    def _B_setup():
        B, Sq, D = 8, 144, 640
        H, Sk, Dh = 32, 512, 128
        return {
            "x": _w((lambda *s: _rng.normal(s) * 0.8)(B, Sq, D)),
            "k_cache": _w((lambda *s: _rng.normal(s) * 0.8)(B, H, Sk, Dh)),
            "v_cache": _w((lambda *s: _rng.normal(s) * 0.05)(B, H, Sk, Dh)),
            "wq": _w((lambda *s: _rng.normal(s) * 0.8)(D, H * Dh) * (D ** -0.5)),
            "wo": _w((lambda *s: _rng.normal(s) * 0.05)(H * Dh, D) * ((H * Dh) ** -0.5)),
        }
    _B_in = _B_setup()

    return {
        "A_x": _A_in["x"],
        "A_k_cache": _A_in["k_cache"],
        "A_v_cache": _A_in["v_cache"],
        "A_wq": _A_in["wq"],
        "A_wo": _A_in["wo"],
        "B_x": _B_in["x"],
        "B_k_cache": _B_in["k_cache"],
        "B_v_cache": _B_in["v_cache"],
        "B_wq": _B_in["wq"],
        "B_wo": _B_in["wo"],
    }

def reference(A_x, A_k_cache, A_v_cache, A_wq, A_wo, B_x, B_k_cache, B_v_cache, B_wq, B_wo):
    def _A_ref(x, k_cache, v_cache, wq, wo):
        B, Sq, D = x.shape
        H, Dh = 32, 128
        q = (lambda x, *d: x.transpose(*d))((x @ wq).reshape(B, Sq, H, Dh), 0, 2, 1, 3)
        scores = jnp.einsum("bhqd,bhkd->bhqk", q, k_cache) * (Dh ** -0.5)
        p = _softmax(scores, axis=-1)
        o = jnp.einsum("bhqk,bhkd->bhqd", p, v_cache)
        return (lambda x, *d: x.transpose(*d))(o, 0, 2, 1, 3).reshape(B, Sq, H * Dh) @ wo

    def _B_ref(x, k_cache, v_cache, wq, wo):
        B, Sq, D = x.shape
        H, Dh = 32, 128
        q = (lambda x, *d: x.transpose(*d))((x @ wq).reshape(B, Sq, H, Dh), 0, 2, 1, 3)
        scores = jnp.einsum("bhqd,bhkd->bhqk", q, k_cache) * (Dh ** -0.5)
        p = _softmax(scores, axis=-1)
        o = jnp.einsum("bhqk,bhkd->bhqd", p, v_cache)
        return (lambda x, *d: x.transpose(*d))(o, 0, 2, 1, 3).reshape(B, Sq, H * Dh) @ wo

    a = _A_ref(A_x, A_k_cache, A_v_cache, A_wq, A_wo)
    b = _B_ref(B_x, B_k_cache, B_v_cache, B_wq, B_wo)
    return jnp.concatenate([a, b], axis=-1)
```

```python
import jax
import jax.numpy as jnp
import jax.experimental.pallas as pl
import jax.experimental.pallas.tpu as pltpu

_LOG2E = 1.4426950408889634
_NT = (((1,), (1,)), ((), ()))
_DH = 128


def _recip(l):
    r = pltpu.reciprocal(l, approx=True)
    return r * (2.0 - l * r)


@jax.jit
def pallas_concat_heads__mha_block_cached__mha_block_cached__near_ridge_kernel(
    A_x: jax.Array,
    A_k_cache: jax.Array,
    A_v_cache: jax.Array,
    A_wq: jax.Array,
    A_wo: jax.Array,
    B_x: jax.Array,
    B_k_cache: jax.Array,
    B_v_cache: jax.Array,
    B_wq: jax.Array,
    B_wo: jax.Array,
):
    B, SQ, D = A_x.shape
    _, H, SK, DH = A_k_cache.shape
    M = B * SQ
    U = 2 * B
    c = (DH ** -0.5) * _LOG2E

    def kernel(xa, ka, va, wqa, woa, xb, kb, vb, wqb, wob, o_ref, acc_a, acc_b):
        h = pl.program_id(0)
        X = (xa, xb); K = (ka, kb); V = (va, vb); WQ = (wqa, wqb); WO = (woa, wob); ACC = (acc_a, acc_b)

        @pl.when(h == 0)
        def _():
            acc_a[...] = jnp.zeros_like(acc_a)
            acc_b[...] = jnp.zeros_like(acc_b)

        qv, sv, ov = {}, {}, {}

        def st_q(u):
            s, b = divmod(u, B)
            q = jnp.dot(X[s][b * SQ:(b + 1) * SQ, :], WQ[s][...], preferred_element_type=jnp.float32)
            qv[u] = q.astype(jnp.bfloat16)

        def st_k(u):
            s, b = divmod(u, B)
            sv[u] = jax.lax.dot_general(qv.pop(u), K[s][b, 0], _NT, preferred_element_type=jnp.float32)

        def st_p(u):
            s, b = divmod(u, B)
            sc = sv.pop(u)
            m = jnp.max(sc, axis=-1, keepdims=True)
            p = jnp.exp2((sc - m) * c)
            l = jnp.sum(p, axis=-1, keepdims=True)
            o = jnp.dot(p.astype(jnp.bfloat16), V[s][b, 0], preferred_element_type=jnp.float32)
            ov[u] = (o * _recip(l)).astype(jnp.bfloat16)

        def st_o(u):
            s, b = divmod(u, B)
            r = jnp.dot(ov.pop(u), WO[s][...], preferred_element_type=jnp.float32)
            ACC[s][b * SQ:(b + 1) * SQ, :] += r

        for t in range(-2, U + 1):
            for f, off in ((st_q, 2), (st_k, 1), (st_p, 0), (st_o, -1)):
                if 0 <= t + off < U:
                    f(t + off)

        @pl.when(h == H - 1)
        def _():
            o_ref[:, :D] = acc_a[...].astype(jnp.bfloat16)
            o_ref[:, D:] = acc_b[...].astype(jnp.bfloat16)

    xs = pl.BlockSpec((M, D), lambda h: (0, 0))
    kv = pl.BlockSpec((B, 1, SK, DH), lambda h: (0, h, 0, 0))
    wq = pl.BlockSpec((D, DH), lambda h: (0, h))
    wo = pl.BlockSpec((DH, D), lambda h: (h, 0))
    out = pl.pallas_call(
        kernel,
        grid=(H,),
        in_specs=[xs, kv, kv, wq, wo] * 2,
        out_specs=pl.BlockSpec((M, 2 * D), lambda h: (0, 0)),
        out_shape=jax.ShapeDtypeStruct((M, 2 * D), jnp.bfloat16),
        scratch_shapes=[pltpu.VMEM((M, D), jnp.float32)] * 2,
        compiler_params=pltpu.CompilerParams(
            dimension_semantics=("arbitrary",), vmem_limit_bytes=100 * 1024 * 1024),
    )(A_x.reshape(M, D), A_k_cache, A_v_cache, A_wq, A_wo,
      B_x.reshape(M, D), B_k_cache, B_v_cache, B_wq, B_wo)
    return out.reshape(B, SQ, 2 * D)
```

```python
import jax
import jax.numpy as jnp
from jax import lax
import jax.experimental.pallas as pl
import jax.experimental.pallas.tpu as pltpu

_LOG2E = 1.4426950408889634
_NT = (((1,), (1,)), ((), ()))

_RING = 12
_AHEAD = 9
_PRE = 8
_PEEL = (2, 6)
_CQ = 8
_XSPLIT = 2
_FIRST = 2
_HP = 2
_TAIL = (1, 1)


def _recip(l):
    r = pltpu.reciprocal(l, approx=True)
    return r * (2.0 - l * r)


@jax.jit
def pallas_concat_heads__mha_block_cached__mha_block_cached__near_ridge_kernel(
    A_x: jax.Array,
    A_k_cache: jax.Array,
    A_v_cache: jax.Array,
    A_wq: jax.Array,
    A_wo: jax.Array,
    B_x: jax.Array,
    B_k_cache: jax.Array,
    B_v_cache: jax.Array,
    B_wq: jax.Array,
    B_wo: jax.Array,
):
    B, SQ, D = A_x.shape
    _, H, SK, DH = A_k_cache.shape
    M = B * SQ
    UH = 2 * B
    R = _RING
    scale = (DH ** -0.5) * _LOG2E
    bf = jnp.bfloat16

    chunks = []
    h0 = 0
    for n in _PEEL:
        chunks.append((0, h0, n))
        h0 += n
    npeel = len(chunks)
    h_loop0 = h0
    assert (H - h0) % _CQ == 0 and H % _CQ == 0 and B % _XSPLIT == 0
    chunks += [(0, h, _CQ) for h in range(h0, H, _CQ)]
    first_b = len(chunks)
    chunks += [(1, h, _CQ) for h in range(0, H, _CQ)]
    nch = len(chunks)
    kv_at = [min(k + 1, nch - 1) for k in range(_PRE)]
    BX = B // _XSPLIT
    n_loop = (H - _FIRST - sum(_TAIL)) // _HP
    assert _FIRST + n_loop * _HP + sum(_TAIL) == H and n_loop > 0
    maxi = _HP

    def last_issue(a):
        return min(a + R - 2, a + _AHEAD, H - 1)

    issued = max(_PRE, min(last_issue(0), _PRE + 1) + 1)
    a = 0
    for n in (_FIRST,) + (_HP,) * n_loop + _TAIL:
        assert issued >= a + n
        a += n
        nxt = max(issued, last_issue(a) + 1)
        assert nxt - issued <= maxi or a <= _FIRST
        issued = nxt
    assert issued == H and R >= 2 * _HP + 1 and _PRE <= R - 1

    def kernel(xa, ka, va, wqa, woa, xb, kb, vb, wqb, wob, out_hbm,
               x_buf, wq_buf, q_buf, kv_buf, wo_buf, acc, s_c, o_c, out_buf,
               x_sem, wq_sem, kv_sem, wo_sem, out_sem):
        K = (ka, kb)
        V = (va, vb)
        WQ = (wqa, wqb)
        WO = (woa, wob)

        def aligned(x, m):
            return x if isinstance(x, int) else pl.multiple_of(x, m)

        def xa_dma(p):
            rows = pl.ds(p * BX * SQ, BX * SQ)
            return pltpu.make_async_copy(xa.at[rows], x_buf.at[0, rows], x_sem.at[p])

        def xb_dma():
            return pltpu.make_async_copy(xb, x_buf.at[1], x_sem.at[_XSPLIT])

        def wq_dma(ci):
            s, h, n = chunks[ci]
            cols = pl.ds(h * DH, n * DH)
            return pltpu.make_async_copy(
                WQ[s].at[:, cols], wq_buf.at[s, :, cols], wq_sem.at[ci])

        def head_start(h, slot):
            rows = pl.ds(aligned(h * DH, DH), DH)
            for s in range(2):
                pltpu.make_async_copy(K[s].at[:, h], kv_buf.at[slot, 0, s], kv_sem.at[slot]).start()
                pltpu.make_async_copy(V[s].at[:, h], kv_buf.at[slot, 1, s], kv_sem.at[slot]).start()
                pltpu.make_async_copy(WO[s].at[rows, :], wo_buf.at[slot, s], wo_sem.at[slot]).start()

        def head_wait(slot):
            pltpu.make_async_copy(kv_buf.at[slot], kv_buf.at[slot], kv_sem.at[slot]).wait()
            pltpu.make_async_copy(wo_buf.at[slot], wo_buf.at[slot], wo_sem.at[slot]).wait()

        def out_dma(u):
            s, b = divmod(u, B)
            return pltpu.make_async_copy(
                out_buf.at[u], out_hbm.at[pl.ds(b * SQ, SQ), pl.ds(s * D, D)], out_sem.at[u])

        def starts_after(ci):
            todo = []
            nx = ci + 2
            if nx < nch:
                if nx == first_b:
                    todo.append(lambda: xb_dma().start())
                todo.append(lambda: wq_dma(nx).start())
            for k, at in enumerate(kv_at):
                if at == ci:
                    todo.append(lambda k=k: head_start(k, k % R))
            return todo

        def q_chunk(s, h, n, b0=0, b1=B):
            w = wq_buf.at[s, :, pl.ds(aligned(h * DH, DH), n * DH)]
            for b in range(b0, b1):
                rows = slice(b * SQ, (b + 1) * SQ)
                q = jnp.dot(x_buf[s, rows, :], w[...], preferred_element_type=jnp.float32)
                q = q.astype(bf)
                for j in range(n):
                    q_buf[s, h + j, rows, :] = q[:, j * DH:(j + 1) * DH]

        xa_dma(0).start()
        wq_dma(0).start()
        for p in range(1, _XSPLIT):
            xa_dma(p).start()
        wq_dma(1).start()
        acc[...] = jnp.zeros_like(acc)

        for ci in range(npeel):
            wq_dma(ci).wait()
            if ci == 0:
                for p in range(_XSPLIT):
                    xa_dma(p).wait()
                    if p == 0:
                        for f in starts_after(ci):
                            f()
                    q_chunk(*chunks[ci], b0=p * BX, b1=(p + 1) * BX)
            else:
                for f in starts_after(ci):
                    f()
                q_chunk(*chunks[ci])

        n_a = first_b - npeel

        def phase0_body(g, carry):
            in_b = g >= n_a
            s = in_b.astype(jnp.int32)
            h = jnp.where(in_b, (g - n_a) * _CQ, h_loop0 + g * _CQ)
            cols = pl.ds(pl.multiple_of(h * DH, DH), _CQ * DH)
            pltpu.make_async_copy(
                wq_buf.at[s, :, cols], wq_buf.at[s, :, cols], wq_sem.at[g + npeel]).wait()

            @pl.when(g == n_a)
            def _():
                xb_dma().wait()

            for ci in range(npeel, nch):
                todo = starts_after(ci)
                if todo:
                    @pl.when(g == ci - npeel)
                    def _():
                        for f in todo:
                            f()
            q_chunk(s, h, _CQ)
            return carry

        lax.fori_loop(0, nch - npeel, phase0_body, 0)

        scores, outs = {}, {}

        def locate(r, hbase, slots):
            j, u = divmod(r, UH)
            s, b = divmod(u, B)
            return slots[j], hbase + j, s, b, u

        def stage_k(r, hbase, slots):
            slot, h, s, b, _ = locate(r, hbase, slots)
            q = q_buf[s, h, b * SQ:(b + 1) * SQ, :]
            scores[r] = lax.dot_general(
                q, kv_buf[slot, 0, s, b], _NT, preferred_element_type=jnp.float32)

        def stage_p(r, hbase, slots):
            slot, _, s, b, _ = locate(r, hbase, slots)
            sc = scores.pop(r)
            m = jnp.max(sc, axis=-1, keepdims=True)
            p = jnp.exp2((sc - m) * scale)
            l = jnp.sum(p, axis=-1, keepdims=True)
            o = jnp.dot(p.astype(bf), kv_buf[slot, 1, s, b], preferred_element_type=jnp.float32)
            outs[r] = (o * _recip(l)).astype(bf)

        def stage_o(r, hbase, slots, final):
            slot, _, s, b, u = locate(r, hbase, slots)
            res = jnp.dot(outs.pop(r), wo_buf[slot, s], preferred_element_type=jnp.float32)
            rows = slice(b * SQ, (b + 1) * SQ)
            if final:
                out_buf[u] = (acc[s, rows, :] + res).astype(bf)
                out_dma(u).start()
            else:
                acc[s, rows, :] += res

        def wrap(x):
            return jnp.where(x >= R, x - R, x)

        n_issued = [_PRE]

        def segment(hbase, n, is_first=False, is_last=False, dyn=None,
                    carry_in=False, carry_out=False):
            if dyn is None:
                slots = {j: (hbase + j) % R for j in range(-1, n)}
            else:
                iss, sb, isl = dyn
                slots = {j: (sb if j == 0 else wrap(sb + j)) for j in range(n)}
                slots[-1] = wrap(sb + (R - 1))
            for j in range(n):
                head_wait(slots[j])
            if carry_in:
                scores[-1] = s_c[...]
                outs[-2] = o_c[...]
            un = n * UH
            for t in range(un + 2 if is_last else un):
                if t < un:
                    stage_k(t, hbase, slots)
                if t - 1 < un and (t >= 1 or not is_first):
                    stage_p(t - 1, hbase, slots)
                if t >= 2 or not is_first:
                    stage_o(t - 2, hbase, slots, is_last and t - 2 >= un - UH)
            if not is_last:
                scores[-1] = scores.pop(un - 1)
                outs[-2] = outs.pop(un - 2)
            a2 = hbase + n
            new_iss = None
            if dyn is None:
                for k in range(n_issued[0], last_issue(a2) + 1):
                    head_start(k, k % R)
                n_issued[0] = max(n_issued[0], last_issue(a2) + 1)
            else:
                hi = jnp.minimum(a2 + min(R - 2, _AHEAD), H - 1)
                for j in range(maxi):
                    nsl = isl if j == 0 else wrap(isl + j)

                    @pl.when(iss + j <= hi)
                    def _():
                        head_start(iss + j, nsl)
                new_iss = jnp.maximum(iss, hi + 1)
            if carry_out:
                s_c[...] = scores.pop(-1)
                o_c[...] = outs.pop(-2)
            return new_iss

        for k in range(_PRE, min(last_issue(0), _PRE + 1) + 1):
            head_start(k, k % R)
            n_issued[0] = k + 1

        segment(0, _FIRST, is_first=True, carry_out=True)

        def phase1_body(i, dyn):
            iss, sb, isl = dyn
            new_iss = segment(_FIRST + i * _HP, _HP, dyn=dyn, carry_in=True, carry_out=True)
            return new_iss, wrap(sb + _HP), wrap(isl + (new_iss - iss))

        lax.fori_loop(0, n_loop, phase1_body,
                      (jnp.int32(n_issued[0]), jnp.int32(_FIRST % R), jnp.int32(n_issued[0] % R)))
        hb = _FIRST + n_loop * _HP
        n_issued[0] = max(n_issued[0], last_issue(hb) + 1)

        for i, n in enumerate(_TAIL):
            segment(hb, n, is_last=(i == len(_TAIL) - 1), carry_in=(i == 0))
            hb += n

        for u in range(UH):
            out_dma(u).wait()

    any_spec = pl.BlockSpec(memory_space=pl.ANY)
    out = pl.pallas_call(
        kernel,
        in_specs=[any_spec] * 10,
        out_specs=any_spec,
        out_shape=jax.ShapeDtypeStruct((M, 2 * D), bf),
        scratch_shapes=[
            pltpu.VMEM((2, M, D), bf),
            pltpu.VMEM((2, D, H * DH), bf),
            pltpu.VMEM((2, H, M, DH), bf),
            pltpu.VMEM((R, 2, 2, B, SK, DH), bf),
            pltpu.VMEM((R, 2, DH, D), bf),
            pltpu.VMEM((2, M, D), jnp.float32),
            pltpu.VMEM((SQ, SK), jnp.float32),
            pltpu.VMEM((SQ, DH), bf),
            pltpu.VMEM((UH, SQ, D), bf),
            pltpu.SemaphoreType.DMA((_XSPLIT + 1,)),
            pltpu.SemaphoreType.DMA((nch,)),
            pltpu.SemaphoreType.DMA((R,)),
            pltpu.SemaphoreType.DMA((R,)),
            pltpu.SemaphoreType.DMA((UH,)),
        ],
        compiler_params=pltpu.CompilerParams(
            vmem_limit_bytes=124 * 1024 * 1024, disable_bounds_checks=True),
    )(A_x.reshape(M, D), A_k_cache, A_v_cache, A_wq, A_wo,
      B_x.reshape(M, D), B_k_cache, B_v_cache, B_wq, B_wo)
    return out.reshape(B, SQ, 2 * D)
```

```python
import jax
import jax.numpy as jnp
from jax import lax
import jax.experimental.pallas as pl
import jax.experimental.pallas.tpu as pltpu

_LOG2E = 1.4426950408889634
_NT = (((1,), (1,)), ((), ()))

_RING = 8
_PEEL = (2, 6)
_CQ = 8
_XSPLIT = 2
_HP = 3


def _recip(l):
    r = pltpu.reciprocal(l, approx=True)
    return r * (2.0 - l * r)


@jax.jit
def pallas_concat_heads__mha_block_cached__mha_block_cached__near_ridge_kernel(
    A_x: jax.Array,
    A_k_cache: jax.Array,
    A_v_cache: jax.Array,
    A_wq: jax.Array,
    A_wo: jax.Array,
    B_x: jax.Array,
    B_k_cache: jax.Array,
    B_v_cache: jax.Array,
    B_wq: jax.Array,
    B_wo: jax.Array,
):
    B, SQ, D = A_x.shape
    _, H, SK, DH = A_k_cache.shape
    M = B * SQ
    UH = 2 * B
    R = _RING
    scale = (DH ** -0.5) * _LOG2E
    bf = jnp.bfloat16

    chunks = []
    h0 = 0
    for n in _PEEL:
        chunks.append((0, h0, n))
        h0 += n
    npeel = len(chunks)
    h_loop0 = h0
    chunks += [(0, h, _CQ) for h in range(h0, H, _CQ)]
    first_b = len(chunks)
    chunks += [(1, h, _CQ) for h in range(0, H, _CQ)]
    nch = len(chunks)
    n_a = first_b - npeel
    n_pre = R - 1
    BX = B // _XSPLIT
    n_loop = (H - 2) // _HP
    assert npeel == 2 and (H - h_loop0) % _CQ == 0 and H % _CQ == 0 and B % _XSPLIT == 0
    assert n_pre <= nch - npeel and n_loop * _HP == H - 2 and R <= H

    def kernel(xa, ka, va, wqa, woa, xb, kb, vb, wqb, wob, out_hbm,
               x_buf, wq_buf, q_buf, kv_buf, wo_buf, acc, s_c, o_c, out_buf,
               x_sem, wq_sem, kv_sem, wo_sem, out_sem):
        K = (ka, kb)
        V = (va, vb)
        WQ = (wqa, wqb)
        WO = (woa, wob)

        def aligned(x, m):
            return x if isinstance(x, int) else pl.multiple_of(x, m)

        def xa_dma(p):
            rows = pl.ds(p * BX * SQ, BX * SQ)
            return pltpu.make_async_copy(xa.at[rows], x_buf.at[0, rows], x_sem.at[p])

        def xb_dma():
            return pltpu.make_async_copy(xb, x_buf.at[1], x_sem.at[_XSPLIT])

        def wq_dma(ci):
            s, h, n = chunks[ci]
            cols = pl.ds(h * DH, n * DH)
            return pltpu.make_async_copy(
                WQ[s].at[:, cols], wq_buf.at[s, :, cols], wq_sem.at[2 if ci == 0 else ci])

        def head_start(h, slot):
            rows = pl.ds(aligned(h * DH, DH), DH)
            for s in range(2):
                pltpu.make_async_copy(K[s].at[:, h], kv_buf.at[slot, 0, s], kv_sem.at[slot]).start()
                pltpu.make_async_copy(V[s].at[:, h], kv_buf.at[slot, 1, s], kv_sem.at[slot]).start()
                pltpu.make_async_copy(WO[s].at[rows, :], wo_buf.at[slot, s], wo_sem.at[slot]).start()

        def head_wait(slot):
            pltpu.make_async_copy(kv_buf.at[slot], kv_buf.at[slot], kv_sem.at[slot]).wait()
            pltpu.make_async_copy(wo_buf.at[slot], wo_buf.at[slot], wo_sem.at[slot]).wait()

        def out_dma(u):
            s, b = divmod(u, B)
            return pltpu.make_async_copy(
                out_buf.at[u], out_hbm.at[pl.ds(b * SQ, SQ), pl.ds(s * D, D)], out_sem.at[u])

        def starts_after(ci):
            todo = []
            nx = ci + 2
            if nx < nch:
                if nx == first_b:
                    todo.append(lambda: xb_dma().start())
                todo.append(lambda: wq_dma(nx).start())
            k = ci - npeel
            if 0 <= k < n_pre:
                todo.append(lambda: head_start(k, k))
            return todo

        def q_chunk(s, h, n, b0=0, b1=B):
            w = wq_buf.at[s, :, pl.ds(aligned(h * DH, DH), n * DH)]
            for b in range(b0, b1):
                rows = slice(b * SQ, (b + 1) * SQ)
                q = jnp.dot(x_buf[s, rows, :], w[...], preferred_element_type=jnp.float32)
                q = q.astype(bf)
                for j in range(n):
                    q_buf[s, h + j, rows, :] = q[:, j * DH:(j + 1) * DH]

        xa_dma(0).start()
        wq_dma(0).start()
        for p in range(1, _XSPLIT):
            xa_dma(p).start()
        wq_dma(1).start()

        def zero_body(i, carry):
            acc[:, pl.ds(pl.multiple_of(i * SQ, SQ), SQ), :] = jnp.zeros((2, SQ, D), jnp.float32)
            return carry

        lax.fori_loop(0, B, zero_body, 0)

        for ci in range(npeel):
            wq_dma(ci).wait()
            if ci == 0:
                for p in range(_XSPLIT):
                    xa_dma(p).wait()
                    if p == 0:
                        for f in starts_after(ci):
                            f()
                    q_chunk(*chunks[ci], b0=p * BX, b1=(p + 1) * BX)
            else:
                for f in starts_after(ci):
                    f()
                q_chunk(*chunks[ci])

        def phase0_body(g, carry):
            in_b = g >= n_a
            s = in_b.astype(jnp.int32)
            h = jnp.where(in_b, (g - n_a) * _CQ, h_loop0 + g * _CQ)
            cols = pl.ds(pl.multiple_of(h * DH, DH), _CQ * DH)
            pltpu.make_async_copy(
                wq_buf.at[s, :, cols], wq_buf.at[s, :, cols], wq_sem.at[g + npeel]).wait()

            @pl.when(g == n_a)
            def _():
                xb_dma().wait()

            for ci in range(npeel, nch):
                todo = starts_after(ci)
                if todo:
                    @pl.when(g == ci - npeel)
                    def _():
                        for f in todo:
                            f()
            q_chunk(s, h, _CQ)
            return carry

        lax.fori_loop(0, nch - npeel, phase0_body, 0)

        scores, outs = {}, {}

        def locate(r, hbase, slots):
            j, u = divmod(r, UH)
            s, b = divmod(u, B)
            return slots[j], hbase + j, s, b, u

        def stage_k(r, hbase, slots):
            slot, h, s, b, _ = locate(r, hbase, slots)
            q = q_buf[s, h, b * SQ:(b + 1) * SQ, :]
            scores[r] = lax.dot_general(
                q, kv_buf[slot, 0, s, b], _NT, preferred_element_type=jnp.float32)

        def stage_p(r, hbase, slots):
            slot, _, s, b, _ = locate(r, hbase, slots)
            sc = scores.pop(r)
            m = jnp.max(sc, axis=-1, keepdims=True)
            p = jnp.exp2((sc - m) * scale)
            l = jnp.sum(p, axis=-1, keepdims=True)
            o = jnp.dot(p.astype(bf), kv_buf[slot, 1, s, b], preferred_element_type=jnp.float32)
            outs[r] = (o * _recip(l)).astype(bf)

        def stage_o(r, hbase, slots, final):
            slot, _, s, b, u = locate(r, hbase, slots)
            res = jnp.dot(outs.pop(r), wo_buf[slot, s], preferred_element_type=jnp.float32)
            rows = slice(b * SQ, (b + 1) * SQ)
            if final:
                out_buf[u] = (acc[s, rows, :] + res).astype(bf)
                out_dma(u).start()
            else:
                acc[s, rows, :] += res

        def next_slot(x):
            return jnp.where(x >= R - 1, x - (R - 1), x + 1)

        def segment(hbase, n, is_first=False, is_last=False, slot0=None):
            if slot0 is None:
                slots = {j: (hbase + j) % R for j in range(-1, n)}
            else:
                slots = {-1: jnp.where(slot0 >= 1, slot0 - 1, R - 1), 0: slot0}
                for j in range(1, n):
                    slots[j] = next_slot(slots[j - 1])
            if not is_first:
                scores[-1] = s_c[...]
                outs[-2] = o_c[...]
            un = n * UH
            lo = 0 if is_first else -2
            for t in range(un + 2 if is_last else un):
                j, tt = divmod(t, UH)
                if tt == 0 and t < un:
                    head_wait(slots[j])
                if t < un:
                    stage_k(t, hbase, slots)
                if lo <= t - 1 < un:
                    stage_p(t - 1, hbase, slots)
                if lo <= t - 2:
                    stage_o(t - 2, hbase, slots, is_last and t - 2 >= un - UH)
                if tt == 1 and t < un:
                    done = hbase + j - 1
                    if isinstance(done, int):
                        if done >= 0 and done + R < H:
                            head_start(done + R, slots[j - 1])
                    else:
                        @pl.when(done + R < H)
                        def _():
                            head_start(done + R, slots[j - 1])
            if not is_last:
                s_c[...] = scores.pop(un - 1)
                o_c[...] = outs.pop(un - 2)

        for k in range(n_pre, R):
            head_start(k, k)

        segment(0, 1, is_first=True)

        def phase1_body(i, slot0):
            segment(1 + i * _HP, _HP, slot0=slot0)
            for _ in range(_HP):
                slot0 = next_slot(slot0)
            return slot0

        lax.fori_loop(0, n_loop, phase1_body, jnp.int32(1 % R))

        segment(H - 1, 1, is_last=True)

        for u in range(UH):
            out_dma(u).wait()

    any_spec = pl.BlockSpec(memory_space=pl.ANY)
    out = pl.pallas_call(
        kernel,
        in_specs=[any_spec] * 10,
        out_specs=any_spec,
        out_shape=jax.ShapeDtypeStruct((M, 2 * D), bf),
        scratch_shapes=[
            pltpu.VMEM((2, M, D), bf),
            pltpu.VMEM((2, D, H * DH), bf),
            pltpu.VMEM((2, H, M, DH), bf),
            pltpu.VMEM((R, 2, 2, B, SK, DH), bf),
            pltpu.VMEM((R, 2, DH, D), bf),
            pltpu.VMEM((2, M, D), jnp.float32),
            pltpu.VMEM((SQ, SK), jnp.float32),
            pltpu.VMEM((SQ, DH), bf),
            pltpu.VMEM((UH, SQ, D), bf),
            pltpu.SemaphoreType.DMA((_XSPLIT + 1,)),
            pltpu.SemaphoreType.DMA((nch,)),
            pltpu.SemaphoreType.DMA((R,)),
            pltpu.SemaphoreType.DMA((R,)),
            pltpu.SemaphoreType.DMA((UH,)),
        ],
        compiler_params=pltpu.CompilerParams(
            vmem_limit_bytes=110 * 1024 * 1024,
            disable_bounds_checks=True,
            flags={"XLA_TPU_RESCHEDULE_DMA_DONES": True}),
    )(A_x.reshape(M, D), A_k_cache, A_v_cache, A_wq, A_wo,
      B_x.reshape(M, D), B_k_cache, B_v_cache, B_wq, B_wo)
    return out.reshape(B, SQ, 2 * D)
```

```python
import jax
import jax.numpy as jnp
from jax import lax
import jax.experimental.pallas as pl
import jax.experimental.pallas.tpu as pltpu

_LOG2E = 1.4426950408889634
_NT = (((1,), (1,)), ((), ()))

_RING = 8
_PEEL = (3, 2, 3)
_CQ = 8
_XD = 4
_HP = 3


def _recip(l):
    r = pltpu.reciprocal(l, approx=True)
    return r * (2.0 - l * r)


@jax.jit
def pallas_concat_heads__mha_block_cached__mha_block_cached__near_ridge_kernel(
    A_x: jax.Array,
    A_k_cache: jax.Array,
    A_v_cache: jax.Array,
    A_wq: jax.Array,
    A_wo: jax.Array,
    B_x: jax.Array,
    B_k_cache: jax.Array,
    B_v_cache: jax.Array,
    B_wq: jax.Array,
    B_wo: jax.Array,
):
    B, SQ, D = A_x.shape
    _, H, SK, DH = A_k_cache.shape
    M = B * SQ
    UH = 2 * B
    R = _RING
    scale = (DH ** -0.5) * _LOG2E
    bf = jnp.bfloat16

    chunks = []
    h0 = 0
    for n in _PEEL:
        chunks.append((0, h0, n))
        h0 += n
    npeel = len(chunks)
    h_loop0 = h0
    chunks += [(0, h, _CQ) for h in range(h0, H, _CQ)]
    first_b = len(chunks)
    chunks += [(1, h, _CQ) for h in range(0, H, _CQ)]
    nch = len(chunks)
    n_a = first_b - npeel
    n_pre = R - 1
    n_loop = (H - 2) // _HP
    assert npeel == 3 and (H - h_loop0) % _CQ == 0 and H % _CQ == 0 and _XD in (3, 4)
    assert n_pre <= nch - npeel and n_loop * _HP == H - 2 and R <= H

    w1_after, w2_after = B - _XD, B - _XD + 2
    x_slot = {w1_after % _XD: 3, w2_after % _XD: 4}
    for j in range(_XD):
        if j not in x_slot:
            x_slot[j] = len(x_slot) - 2
    wq_slot = {0: 2, 1: 3, 2: 4, **{ci: ci for ci in range(3, nch)}}

    def kernel(xa, ka, va, wqa, woa, xb, kb, vb, wqb, wob, out_hbm,
               x_buf, wq_buf, q_buf, kv_buf, wo_buf, acc, s_c, o_c, out_buf,
               xb_sem, wq_sem, kv_sem, wo_sem, out_sem):
        K = (ka, kb)
        V = (va, vb)
        WQ = (wqa, wqb)
        WO = (woa, wob)

        def aligned(x, m):
            return x if isinstance(x, int) else pl.multiple_of(x, m)

        def xa_dma(p):
            rows = pl.ds(p * SQ, SQ)
            return pltpu.make_async_copy(
                xa.at[rows], x_buf.at[0, rows], wq_sem.at[x_slot[p % _XD]])

        def xb_dma():
            return pltpu.make_async_copy(xb, x_buf.at[1], xb_sem.at[0])

        def wq_dma(ci):
            s, h, n = chunks[ci]
            cols = pl.ds(h * DH, n * DH)
            return pltpu.make_async_copy(
                WQ[s].at[:, cols], wq_buf.at[s, :, cols], wq_sem.at[wq_slot[ci]])

        def head_start(h, slot):
            rows = pl.ds(aligned(h * DH, DH), DH)
            for s in range(2):
                pltpu.make_async_copy(K[s].at[:, h], kv_buf.at[slot, 0, s], kv_sem.at[slot]).start()
                pltpu.make_async_copy(V[s].at[:, h], kv_buf.at[slot, 1, s], kv_sem.at[slot]).start()
                pltpu.make_async_copy(WO[s].at[rows, :], wo_buf.at[slot, s], wo_sem.at[slot]).start()

        def head_wait(slot):
            pltpu.make_async_copy(kv_buf.at[slot], kv_buf.at[slot], kv_sem.at[slot]).wait()
            pltpu.make_async_copy(wo_buf.at[slot], wo_buf.at[slot], wo_sem.at[slot]).wait()

        def out_dma(u):
            s, b = divmod(u, B)
            return pltpu.make_async_copy(
                out_buf.at[u], out_hbm.at[pl.ds(b * SQ, SQ), pl.ds(s * D, D)], out_sem.at[u])

        def starts_after(ci):
            todo = []
            nx = ci + 2
            if nx < nch:
                if nx == first_b:
                    todo.append(lambda: xb_dma().start())
                todo.append(lambda: wq_dma(nx).start())
            k = ci - npeel
            if 0 <= k < n_pre:
                todo.append(lambda: head_start(k, k))
            return todo

        def q_chunk(s, h, n, b0=0, b1=B):
            w = wq_buf.at[s, :, pl.ds(aligned(h * DH, DH), n * DH)]
            for b in range(b0, b1):
                rows = slice(b * SQ, (b + 1) * SQ)
                q = jnp.dot(x_buf[s, rows, :], w[...], preferred_element_type=jnp.float32)
                q = q.astype(bf)
                for j in range(n):
                    q_buf[s, h + j, rows, :] = q[:, j * DH:(j + 1) * DH]

        wq_dma(0).start()
        for p in range(_XD):
            xa_dma(p).start()

        def zero_body(i, carry):
            acc[:, pl.ds(pl.multiple_of(i * SQ, SQ), SQ), :] = jnp.zeros((2, SQ, D), jnp.float32)
            return carry

        lax.fori_loop(0, B, zero_body, 0)

        wq_dma(0).wait()
        for p in range(B):
            xa_dma(p).wait()
            if p + _XD < B:
                xa_dma(p + _XD).start()
            if p == w1_after:
                wq_dma(1).start()
            if p == w2_after:
                wq_dma(2).start()
            q_chunk(*chunks[0], b0=p, b1=p + 1)
        for ci in (1, 2):
            wq_dma(ci).wait()
            wq_dma(ci + 2).start()
            q_chunk(*chunks[ci])

        def phase0_body(g, carry):
            in_b = g >= n_a
            s = in_b.astype(jnp.int32)
            h = jnp.where(in_b, (g - n_a) * _CQ, h_loop0 + g * _CQ)
            cols = pl.ds(pl.multiple_of(h * DH, DH), _CQ * DH)
            pltpu.make_async_copy(
                wq_buf.at[s, :, cols], wq_buf.at[s, :, cols], wq_sem.at[g + npeel]).wait()

            @pl.when(g == n_a)
            def _():
                xb_dma().wait()

            for ci in range(npeel, nch):
                todo = starts_after(ci)
                if todo:
                    @pl.when(g == ci - npeel)
                    def _():
                        for f in todo:
                            f()
            q_chunk(s, h, _CQ)
            return carry

        lax.fori_loop(0, nch - npeel, phase0_body, 0)

        scores, outs = {}, {}

        def locate(r, hbase, slots):
            j, u = divmod(r, UH)
            s, b = divmod(u, B)
            return slots[j], hbase + j, s, b, u

        def stage_k(r, hbase, slots):
            slot, h, s, b, _ = locate(r, hbase, slots)
            q = q_buf[s, h, b * SQ:(b + 1) * SQ, :]
            scores[r] = lax.dot_general(
                q, kv_buf[slot, 0, s, b], _NT, preferred_element_type=jnp.float32)

        def stage_p(r, hbase, slots):
            slot, _, s, b, _ = locate(r, hbase, slots)
            sc = scores.pop(r)
            m = jnp.max(sc, axis=-1, keepdims=True)
            p = jnp.exp2((sc - m) * scale)
            l = jnp.sum(p, axis=-1, keepdims=True)
            o = jnp.dot(p.astype(bf), kv_buf[slot, 1, s, b], preferred_element_type=jnp.float32)
            outs[r] = (o * _recip(l)).astype(bf)

        def stage_o(r, hbase, slots, final):
            slot, _, s, b, u = locate(r, hbase, slots)
            res = jnp.dot(outs.pop(r), wo_buf[slot, s], preferred_element_type=jnp.float32)
            rows = slice(b * SQ, (b + 1) * SQ)
            if final:
                out_buf[u] = (acc[s, rows, :] + res).astype(bf)
                out_dma(u).start()
            else:
                acc[s, rows, :] += res

        def next_slot(x):
            return jnp.where(x >= R - 1, x - (R - 1), x + 1)

        def segment(hbase, n, is_first=False, is_last=False, slot0=None):
            ahead = 0 if is_last else 1
            if slot0 is None:
                slots = {j: (hbase + j) % R for j in range(-1, n + ahead)}
            else:
                slots = {-1: jnp.where(slot0 >= 1, slot0 - 1, R - 1), 0: slot0}
                for j in range(1, n + ahead):
                    slots[j] = next_slot(slots[j - 1])
            un = n * UH
            if is_first:
                head_wait(slots[0])
                stage_k(0, hbase, slots)
            else:
                scores[0] = s_c[...]
                outs[-2] = o_c[0]
                outs[-1] = o_c[1]
            for t in range(un + 2 if is_last else un):
                j, tt = divmod(t, UH)
                if t >= 2 or not is_first:
                    stage_o(t - 2, hbase, slots, is_last and t - 2 >= un - UH)
                if t + 1 < un + ahead:
                    if tt == UH - 1:
                        head_wait(slots[j + 1])
                    stage_k(t + 1, hbase, slots)
                if t < un:
                    stage_p(t, hbase, slots)
                if tt == 1 and t < un:
                    done = hbase + j - 1
                    if isinstance(done, int):
                        if done >= 0 and done + R < H:
                            head_start(done + R, slots[j - 1])
                    else:
                        @pl.when(done + R < H)
                        def _():
                            head_start(done + R, slots[j - 1])
            if not is_last:
                s_c[...] = scores.pop(un)
                o_c[0] = outs.pop(un - 2)
                o_c[1] = outs.pop(un - 1)

        for k in range(n_pre, R):
            head_start(k, k)

        segment(0, 1, is_first=True)

        def phase1_body(i, slot0):
            segment(1 + i * _HP, _HP, slot0=slot0)
            for _ in range(_HP):
                slot0 = next_slot(slot0)
            return slot0

        lax.fori_loop(0, n_loop, phase1_body, jnp.int32(1 % R))

        segment(H - 1, 1, is_last=True)

        for u in range(UH):
            out_dma(u).wait()

    any_spec = pl.BlockSpec(memory_space=pl.ANY)
    out = pl.pallas_call(
        kernel,
        in_specs=[any_spec] * 10,
        out_specs=any_spec,
        out_shape=jax.ShapeDtypeStruct((M, 2 * D), bf),
        scratch_shapes=[
            pltpu.VMEM((2, M, D), bf),
            pltpu.VMEM((2, D, H * DH), bf),
            pltpu.VMEM((2, H, M, DH), bf),
            pltpu.VMEM((R, 2, 2, B, SK, DH), bf),
            pltpu.VMEM((R, 2, DH, D), bf),
            pltpu.VMEM((2, M, D), jnp.float32),
            pltpu.VMEM((SQ, SK), jnp.float32),
            pltpu.VMEM((2, SQ, DH), bf),
            pltpu.VMEM((UH, SQ, D), bf),
            pltpu.SemaphoreType.DMA((1,)),
            pltpu.SemaphoreType.DMA((nch,)),
            pltpu.SemaphoreType.DMA((R,)),
            pltpu.SemaphoreType.DMA((R,)),
            pltpu.SemaphoreType.DMA((UH,)),
        ],
        compiler_params=pltpu.CompilerParams(
            vmem_limit_bytes=110 * 1024 * 1024,
            disable_bounds_checks=True,
            flags={"XLA_TPU_RESCHEDULE_DMA_DONES": True}),
    )(A_x.reshape(M, D), A_k_cache, A_v_cache, A_wq, A_wo,
      B_x.reshape(M, D), B_k_cache, B_v_cache, B_wq, B_wo)
    return out.reshape(B, SQ, 2 * D)
```
